```python
import jax
import jax.numpy as jnp

def _softmax(x, axis=-1):
    return jax.nn.softmax(x, axis=axis)
def _gelu(x):
    return jax.nn.gelu(x, approximate=True)
def _silu(x):
    return jax.nn.silu(x)
def _sigmoid(x):
    return jax.nn.sigmoid(x)
def _layernorm(x, axis=-1, eps=1e-5):
    m = jnp.mean(x, axis=axis, keepdims=True)
    v = jnp.var(x, axis=axis, keepdims=True)
    return (x - m) / jnp.sqrt(v + eps)
def _scatter_add(tgt, idx, src, axis=0):
    return tgt.at[idx].add(src)
def _segment_sum(src, seg, n):
    return jax.ops.segment_sum(src, seg, n)
class _Rng:
    def __init__(self, key):
        self._k = key
    def _next(self):
        self._k, sub = jax.random.split(self._k)
        return sub
    def normal(self, shape):
        return jax.random.normal(self._next(), shape, dtype=jnp.bfloat16)
    def randint(self, lo, hi, shape):
        return jax.random.randint(self._next(), shape, lo, hi, dtype=jnp.int32)
    def uniform(self, shape, lo=0.0, hi=1.0):
        return jax.random.uniform(self._next(), shape, jnp.bfloat16, lo, hi)
    def permutation(self, n):
        return jax.random.permutation(self._next(), n)


kernel_name = 'standalone__modern_conv_block_replknet__vision'

def setup_inputs():
    _rng = _Rng(jax.random.key(int.from_bytes(__import__("os").urandom(4), "little")))
    _w = (lambda a: (lambda t: t.astype(jnp.bfloat16) if jnp.issubdtype(t.dtype, jnp.floating) else t)(jnp.asarray(a)))
    H = W = 512
    C = 96
    K = 3
    return {
        "x": _w((lambda *s: _rng.normal(s) * 0.05)(1, H, W, C)),
        "dw_large": _w((lambda *s: _rng.normal(s) * 0.05)(K, K, C) * (1.0 / K)),
        "dw_small": _w((lambda *s: _rng.normal(s) * 0.05)(5, 5, C) * 0.2),
        "w1": _w((lambda *s: _rng.normal(s) * 0.05)(C, 4 * C) * (C ** -0.5)),
        "w2": _w((lambda *s: _rng.normal(s) * 0.05)(4 * C, C) * ((4 * C) ** -0.5)),
    }

def reference(x, dw_large, dw_small, w1, w2):
    B, H, W, C = x.shape
    Kl = dw_large.shape[0]
    pl = (Kl - 1) // 2
    xpl = jnp.pad(x, ((0,0),(pl,pl),(pl,pl),(0,0)))
    out = jnp.zeros_like(x)
    for i in range(Kl):
        for j in range(Kl):
            out = out + xpl[:, i:i+H, j:j+W, :] * dw_large[i, j][None, None, None, :]
    Ks = dw_small.shape[0]
    ps = (Ks - 1) // 2
    xps = jnp.pad(x, ((0,0),(ps,ps),(ps,ps),(0,0)))
    for i in range(Ks):
        for j in range(Ks):
            out = out + xps[:, i:i+H, j:j+W, :] * dw_small[i, j][None, None, None, :]
    h = _layernorm(out, axis=-1)
    h = _gelu(jnp.einsum('bhwc,ce->bhwe', h, w1))
    h = jnp.einsum('bhwe,ec->bhwc', h, w2)
    return x + h
```

```python
import jax
import jax.numpy as jnp
import jax.experimental.pallas as pl
import jax.experimental.pallas.tpu as pltpu

HB = 32
F32 = jnp.float32


def _kernel(x_ref, top_ref, bot_ref, ds_ref, dl_ref, w1_ref, w2_ref, o_ref,
            xs, cv, wb, w2s):
    i = pl.program_id(0)
    n = pl.num_programs(0)
    C, W = x_ref.shape[1:]
    NT = W // 128

    @pl.when(i == 0)
    def _():
        ds = ds_ref[...]
        dl = dl_ref[...]
        for a in range(5):
            for b in range(5):
                w = ds[:, a * 5 + b:a * 5 + b + 1]
                if 1 <= a <= 3 and 1 <= b <= 3:
                    k = (a - 1) * 3 + b - 1
                    w = w + dl[:, k:k + 1]
                wb[a * 5 + b] = jnp.broadcast_to(w, (C, 128))
        w2s[...] = (w2_ref[...].astype(F32) * 0.5).astype(w2s.dtype)

    xs[0:2] = jnp.where(i > 0, top_ref[...].astype(F32), 0.0)
    xs[HB + 2:HB + 4] = jnp.where(i < n - 1, bot_ref[...].astype(F32), 0.0)

    def cvt(r, _):
        xs[r + 2] = x_ref[r].astype(F32)
    jax.lax.fori_loop(0, HB, cvt, None, unroll=4)

    lane = jax.lax.broadcasted_iota(jnp.int32, (8, 128), 1)

    def conv(h, slot):
        for g in range(C // 8):
            cs = slice(g * 8, g * 8 + 8)
            acc = [None] * NT
            xv = [[xs[h + a, cs, t * 128:(t + 1) * 128] for t in range(NT)]
                  for a in range(5)]
            for b in (2, 0, 4, 1, 3):
                p = []
                ws = [wb[a * 5 + b, cs, :] for a in range(5)]
                for t in range(NT):
                    v = xv[0][t] * ws[0]
                    for a in range(1, 5):
                        v = v + xv[a][t] * ws[a]
                    p.append(v)
                d = b - 2
                if d == 0:
                    acc = p
                    continue
                r = [pltpu.roll(v, (-d) % 128, 1) for v in p]
                for t in range(NT):
                    if d < 0:
                        nb = r[t - 1] if t > 0 else 0.0
                        s = jnp.where(lane < -d, nb, r[t])
                    else:
                        nb = r[t + 1] if t < NT - 1 else 0.0
                        s = jnp.where(lane >= 128 - d, nb, r[t])
                    acc[t] = acc[t] + s
            for t in range(NT):
                cv[slot, cs, t * 128:(t + 1) * 128] = acc[t]

    def mlp(h, slot):
        o = cv[slot]
        m = jnp.sum(o, axis=0, keepdims=True) * (1.0 / C)
        d = o - m
        v = jnp.sum(d * d, axis=0, keepdims=True) * (1.0 / C)
        hn = (d * jax.lax.rsqrt(v + 1e-5)).astype(jnp.bfloat16)
        z = jnp.dot(w1_ref[...], hn, preferred_element_type=F32)
        k0 = 0.7978845608028654
        g = z * (1.0 + jnp.tanh(z * (k0 + (k0 * 0.044715) * (z * z))))
        y = jnp.dot(w2s[...], g.astype(jnp.bfloat16), preferred_element_type=F32)
        o_ref[h] = (xs[h + 2] + y).astype(o_ref.dtype)

    conv(0, 0)

    def body(j, _):
        h = 2 * j
        conv(h + 1, 1)
        mlp(h, 0)
        conv(h + 2, 0)
        mlp(h + 1, 1)
    jax.lax.fori_loop(0, HB // 2 - 1, body, None)
    conv(HB - 1, 1)
    mlp(HB - 2, 0)
    mlp(HB - 1, 1)


@jax.jit
def pallas_standalone__modern_conv_block_replknet__vision_kernel(
    x, dw_large, dw_small, w1, w2):
    _, H, W, C = x.shape
    xt = x[0].transpose(0, 2, 1)
    ds = dw_small.reshape(25, C).T.astype(F32)
    dl = dw_large.reshape(9, C).T.astype(F32)
    nb = H // HB
    full = lambda a: pl.BlockSpec(a.shape, lambda i: (0,) * a.ndim)
    w1t, w2t = w1.T, w2.T
    out = pl.pallas_call(
        _kernel,
        grid=(nb,),
        in_specs=[
            pl.BlockSpec((HB, C, W), lambda i: (i, 0, 0)),
            pl.BlockSpec((2, C, W), lambda i: (jnp.maximum(i * (HB // 2) - 1, 0), 0, 0)),
            pl.BlockSpec((2, C, W), lambda i: (jnp.minimum((i + 1) * (HB // 2), H // 2 - 1), 0, 0)),
            full(ds), full(dl), full(w1t), full(w2t),
        ],
        out_specs=pl.BlockSpec((HB, C, W), lambda i: (i, 0, 0)),
        out_shape=jax.ShapeDtypeStruct((H, C, W), x.dtype),
        scratch_shapes=[
            pltpu.VMEM((HB + 4, C, W), F32),
            pltpu.VMEM((2, C, W), F32),
            pltpu.VMEM((25, C, 128), F32),
            pltpu.VMEM(w2t.shape, w2t.dtype),
        ],
        compiler_params=pltpu.CompilerParams(
            dimension_semantics=("arbitrary",), vmem_limit_bytes=64 << 20),
    )(xt, xt, xt, ds, dl, w1t, w2t)
    return out.transpose(0, 2, 1)[None]
```

```python
import jax
import jax.numpy as jnp
import jax.experimental.pallas as pl
import jax.experimental.pallas.tpu as pltpu

HB = 32
K0 = 0.7978845608028654
S = (K0 * 0.044715) ** (1 / 3)
F32 = jnp.float32


def _kernel(x_ref, top_ref, bot_ref, ds_ref, dl_ref, w1_ref, w2_ref, o_ref,
            xs, cv, wb):
    i = pl.program_id(0)
    n = pl.num_programs(0)
    C, W = x_ref.shape[1:]
    NT = W // 128

    @pl.when(i == 0)
    def _():
        ds = ds_ref[...]
        dl = dl_ref[...]
        for a in range(5):
            for b in range(5):
                w = ds[:, a * 5 + b:a * 5 + b + 1]
                if 1 <= a <= 3 and 1 <= b <= 3:
                    k = (a - 1) * 3 + b - 1
                    w = w + dl[:, k:k + 1]
                wb[a * 5 + b] = jnp.broadcast_to(w, (C, 128))

    xs[0:2] = jnp.where(i > 0, top_ref[...].astype(F32), 0.0)
    xs[HB + 2:HB + 4] = jnp.where(i < n - 1, bot_ref[...].astype(F32), 0.0)

    def cvt(r, _):
        xs[r + 2] = x_ref[r].astype(F32)
    jax.lax.fori_loop(0, HB, cvt, None, unroll=4)

    lane = jax.lax.broadcasted_iota(jnp.int32, (8, 128), 1)

    def conv(h, slot):
        for g in range(C // 8):
            cs = slice(g * 8, g * 8 + 8)
            acc = [None] * NT
            xv = [[xs[h + a, cs, t * 128:(t + 1) * 128] for t in range(NT)]
                  for a in range(5)]
            for b in (2, 0, 4, 1, 3):
                p = []
                ws = [wb[a * 5 + b, cs, :] for a in range(5)]
                for t in range(NT):
                    v = xv[0][t] * ws[0]
                    for a in range(1, 5):
                        v = v + xv[a][t] * ws[a]
                    p.append(v)
                d = b - 2
                if d == 0:
                    acc = p
                    continue
                r = [pltpu.roll(v, (-d) % 128, 1) for v in p]
                for t in range(NT):
                    if d < 0:
                        nb = r[t - 1] if t > 0 else 0.0
                        s = jnp.where(lane < -d, nb, r[t])
                    else:
                        nb = r[t + 1] if t < NT - 1 else 0.0
                        s = jnp.where(lane >= 128 - d, nb, r[t])
                    acc[t] = acc[t] + s
            for t in range(NT):
                cv[slot, cs, t * 128:(t + 1) * 128] = acc[t]

    def mlp(h, slot):
        o = cv[slot]
        m = jnp.sum(o, axis=0, keepdims=True) * (1.0 / C)
        d = o - m
        v = jnp.sum(d * d, axis=0, keepdims=True) * (1.0 / C)
        hn = (d * (jax.lax.rsqrt(v + 1e-5) * S)).astype(jnp.bfloat16)
        z = jnp.dot(w1_ref[...], hn, preferred_element_type=F32)
        g = z * (1.0 + jnp.tanh(z * (K0 / S + z * z)))
        y = jnp.dot(w2_ref[...], g.astype(jnp.bfloat16), preferred_element_type=F32)
        o_ref[h] = (xs[h + 2] + y * (0.5 / S)).astype(o_ref.dtype)

    conv(0, 0)

    def body(j, _):
        h = 2 * j
        mlp(h, 0)
        conv(h + 1, 1)
        mlp(h + 1, 1)
        conv(h + 2, 0)
    jax.lax.fori_loop(0, HB // 2 - 1, body, None, unroll=3)
    conv(HB - 1, 1)
    mlp(HB - 2, 0)
    mlp(HB - 1, 1)


@jax.jit
def pallas_standalone__modern_conv_block_replknet__vision_kernel(
    x, dw_large, dw_small, w1, w2):
    _, H, W, C = x.shape
    xt = x[0].transpose(0, 2, 1)
    ds = dw_small.reshape(25, C).T.astype(F32)
    dl = dw_large.reshape(9, C).T.astype(F32)
    nb = H // HB
    full = lambda a: pl.BlockSpec(a.shape, lambda i: (0,) * a.ndim)
    w1t, w2t = w1.T, w2.T
    out = pl.pallas_call(
        _kernel,
        grid=(nb,),
        in_specs=[
            pl.BlockSpec((HB, C, W), lambda i: (i, 0, 0)),
            pl.BlockSpec((2, C, W), lambda i: (jnp.maximum(i * (HB // 2) - 1, 0), 0, 0)),
            pl.BlockSpec((2, C, W), lambda i: (jnp.minimum((i + 1) * (HB // 2), H // 2 - 1), 0, 0)),
            full(ds), full(dl), full(w1t), full(w2t),
        ],
        out_specs=pl.BlockSpec((HB, C, W), lambda i: (i, 0, 0)),
        out_shape=jax.ShapeDtypeStruct((H, C, W), x.dtype),
        scratch_shapes=[
            pltpu.VMEM((HB + 4, C, W), F32),
            pltpu.VMEM((2, C, W), F32),
            pltpu.VMEM((25, C, 128), F32),
        ],
        compiler_params=pltpu.CompilerParams(
            dimension_semantics=("arbitrary",), vmem_limit_bytes=64 << 20, flags={'XLA_TPU_FORCE_LP_LLO_SCHEDULER': True}),
    )(xt, xt, xt, ds, dl, w1t, w2t)
    return out.transpose(0, 2, 1)[None]
```

```python
import jax
import jax.numpy as jnp
import jax.experimental.pallas as pl
import jax.experimental.pallas.tpu as pltpu

HB = 8
NCH = 2
FLAGS = {'XLA_TPU_FORCE_LP_LLO_SCHEDULER': True}
K0 = 0.7978845608028654
S = (K0 * 0.044715) ** (1 / 3)
F32 = jnp.float32


def _kernel(x_ref, ds_ref, dl_ref, w1_ref, w2_ref, o_ref,
            xs, cv, wb, hs, gs, xb, ob, si, so):
    H, C, W = x_ref.shape
    n = H // HB
    NT = W // 128

    def cin(k):
        return pltpu.make_async_copy(x_ref.at[pl.ds(k * HB, HB)], xb.at[k & 1], si.at[k & 1])

    def cout(k):
        return pltpu.make_async_copy(ob.at[pl.ds((k & 3) * HB, HB)],
                                     o_ref.at[pl.ds(k * HB, HB)], so.at[k & 3])
    cin(0).start()
    for ref in (xs, cv, hs, gs):
        ref[...] = jnp.zeros(ref.shape, ref.dtype)
    if True:
        ds = ds_ref[...]
        dl = dl_ref[...]
        for a in range(5):
            for b in range(5):
                w = ds[:, a * 5 + b:a * 5 + b + 1]
                if 1 <= a <= 3 and 1 <= b <= 3:
                    k = (a - 1) * 3 + b - 1
                    w = w + dl[:, k:k + 1]
                wb[a * 5 + b] = jnp.broadcast_to(w, (C, 128))

    lane = jax.lax.broadcasted_iota(jnp.int32, (8, 128), 1)

    def conv(h, slot, groups):
        for g in groups:
            cs = slice(g * 8, g * 8 + 8)
            acc = [None] * NT
            xv = [[xs[(h + a - 2) & 7, cs, t * 128:(t + 1) * 128] for t in range(NT)]
                  for a in range(5)]
            for b in (2, 0, 4, 1, 3):
                p = []
                ws = [wb[a * 5 + b, cs, :] for a in range(5)]
                for t in range(NT):
                    v = xv[0][t] * ws[0]
                    for a in range(1, 5):
                        v = v + xv[a][t] * ws[a]
                    p.append(v)
                d = b - 2
                if d == 0:
                    acc = p
                    continue
                r = [pltpu.roll(v, (-d) % 128, 1) for v in p]
                for t in range(NT):
                    if d < 0:
                        nb = r[t - 1] if t > 0 else 0.0
                        s = jnp.where(lane < -d, nb, r[t])
                    else:
                        nb = r[t + 1] if t < NT - 1 else 0.0
                        s = jnp.where(lane >= 128 - d, nb, r[t])
                    acc[t] = acc[t] + s
            for t in range(NT):
                cv[slot, cs, t * 128:(t + 1) * 128] = acc[t]

    def norm(slot):
        o = cv[slot]
        m = jnp.sum(o, axis=0, keepdims=True) * (1.0 / C)
        d = o - m
        v = jnp.sum(d * d, axis=0, keepdims=True) * (1.0 / C)
        hs[slot] = (d * (jax.lax.rsqrt(v + 1e-5) * S)).astype(jnp.bfloat16)

    def up(slot, ws):
        z = jnp.dot(w1_ref[...], hs[slot, :, ws], preferred_element_type=F32)
        g = z * (1.0 + jnp.tanh(z * (K0 / S + z * z)))
        gs[slot, :, ws] = g.astype(gs.dtype)

    def down(h, slot, ws):
        y = jnp.dot(w2_ref[...], gs[slot, :, ws], preferred_element_type=F32)
        ob[h & (4 * HB - 1), :, ws] = (xs[h & 7, :, ws] + y * (0.5 / S)).astype(o_ref.dtype)

    def chunk(k, _):
        @pl.when(k < n)
        def _():
            cin(k).wait()

        @pl.when(k + 1 < n)
        def _():
            cin(k + 1).start()

        @pl.when(k == n)
        def _():
            xb[n & 1, 0:8] = jnp.zeros((8, C, W), xb.dtype)

        @pl.when(k >= 3)
        def _():
            cout(k - 3).wait()

        def body(j, _):
            for v in range(8):
                u = v & 1
                r = k * HB + 8 * j + v
                norm(1 - u)
                for c in range(NCH):
                    ws = slice(c * W // NCH, (c + 1) * W // NCH)
                    up(u, ws)
                    down(r - 6, 1 - u, ws)
                    conv(r - 3, u, range(c * 12 // NCH, (c + 1) * 12 // NCH))
                xs[r & 7] = xb[k & 1, 8 * j + v].astype(F32)
        jax.lax.fori_loop(0, jnp.where(k < n, HB // 8, -(-6 // 8)), body, None)

        @pl.when(k >= 1)
        def _():
            cout(k - 1).start()
    jax.lax.fori_loop(0, n + 1, chunk, None)
    cout(n - 2).wait()
    cout(n - 1).wait()


@jax.jit
def pallas_standalone__modern_conv_block_replknet__vision_kernel(
    x, dw_large, dw_small, w1, w2):
    _, H, W, C = x.shape
    xt = x[0].transpose(0, 2, 1)
    ds = dw_small.reshape(25, C).T.astype(F32)
    dl = dw_large.reshape(9, C).T.astype(F32)
    hbm = pl.BlockSpec(memory_space=pl.ANY)
    vm = pl.BlockSpec(memory_space=pltpu.VMEM)
    w1t, w2t = w1.T, w2.T
    out = pl.pallas_call(
        _kernel,
        in_specs=[hbm, vm, vm, vm, vm],
        out_specs=hbm,
        out_shape=jax.ShapeDtypeStruct((H, C, W), x.dtype),
        scratch_shapes=[
            pltpu.VMEM((8, C, W), F32),
            pltpu.VMEM((2, C, W), F32),
            pltpu.VMEM((25, C, 128), F32),
            pltpu.VMEM((2, C, W), x.dtype),
            pltpu.VMEM((2, 4 * C, W), x.dtype),
            pltpu.VMEM((2, HB, C, W), x.dtype),
            pltpu.VMEM((4 * HB, C, W), x.dtype),
            pltpu.SemaphoreType.DMA((2,)),
            pltpu.SemaphoreType.DMA((4,)),
        ],
        compiler_params=pltpu.CompilerParams(
            vmem_limit_bytes=64 << 20, flags=FLAGS),
    )(xt, ds, dl, w1t, w2t)
    return out.transpose(0, 2, 1)[None]
```
